```python
import os as _os
_os.environ.setdefault("JAX_PLATFORMS", "cpu")
import jax
import jax.numpy as jnp

def _softmax(x, axis=-1):
    return jax.nn.softmax(x, axis=axis)
def _gelu(x):
    return jax.nn.gelu(x, approximate=True)
def _silu(x):
    return jax.nn.silu(x)
def _sigmoid(x):
    return jax.nn.sigmoid(x)
def _layernorm(x, axis=-1, eps=1e-5):
    m = jnp.mean(x, axis=axis, keepdims=True)
    v = jnp.var(x, axis=axis, keepdims=True)
    return (x - m) / jnp.sqrt(v + eps)
def _scatter_add(tgt, idx, src, axis=0):
    return tgt.at[idx].add(src)
def _segment_sum(src, seg, n):
    return jax.ops.segment_sum(src, seg, n)
class _Rng:
    def __init__(self, key):
        self._k = key
    def _next(self):
        self._k, sub = jax.random.split(self._k)
        return sub
    def normal(self, shape):
        return jax.random.normal(self._next(), shape, dtype=jnp.bfloat16)
    def randint(self, lo, hi, shape):
        return jax.random.randint(self._next(), shape, lo, hi, dtype=jnp.int32)
    def uniform(self, shape, lo=0.0, hi=1.0):
        return jax.random.uniform(self._next(), shape, jnp.bfloat16, lo, hi)
    def permutation(self, n):
        return jax.random.permutation(self._next(), n)


kernel_name = 'standalone__mha_softmax__near_ridge'

def setup_inputs():
    _rng = _Rng(jax.random.key(int.from_bytes(__import__("os").urandom(4), "little")))
    _w = (lambda a: (lambda t: t.astype(jnp.bfloat16) if jnp.issubdtype(t.dtype, jnp.floating) else t)(jnp.asarray(a)))
    B, H, Sq, Sk, D = 8, 32, 384, 512, 128
    return {
        "q": _w((lambda *s: _rng.normal(s) * 0.4)(B, H, Sq, D)),
        "k": _w((lambda *s: _rng.normal(s) * 0.4)(B, H, Sk, D)),
        "v": _w((lambda *s: _rng.normal(s) * 0.05)(B, H, Sk, D)),
    }

def reference(q, k, v):
    scale = q.shape[-1] ** -0.5
    scores = jnp.einsum("bhqd,bhkd->bhqk", q, k) * scale
    p = _softmax(scores, axis=-1)
    return jnp.einsum("bhqk,bhkd->bhqd", p, v)
```

```python
import jax
import jax.numpy as jnp
from jax import lax
import jax.experimental.pallas as pl
import jax.experimental.pallas.tpu as pltpu

_LOG2E = 1.4426950408889634

_GROUP = 8
_CHUNK = 16
_SWITCH = 13
_LAST = 4


def _attend(q, k, v):
    scale = (q.shape[-1] ** -0.5) * _LOG2E
    s = lax.dot_general(
        q, k, (((1,), (1,)), ((), ())), preferred_element_type=jnp.float32
    )
    m = jnp.max(s, axis=-1, keepdims=True)
    p = jnp.exp2((s - m) * scale)
    l = jnp.sum(p, axis=-1, keepdims=True)
    o = jnp.dot(p.astype(v.dtype), v, preferred_element_type=jnp.float32)
    r = pl.reciprocal(l, approx=True)
    r = r * (2.0 - l * r)
    return o * r


@jax.jit
def pallas_standalone__mha_softmax__near_ridge_kernel(
    q: jax.Array,
    k: jax.Array,
    v: jax.Array,
):
    b, h, sq, d = q.shape
    sk = k.shape[2]
    n = b * h
    nc = n // _CHUNK
    h0 = _SWITCH * _CHUNK

    def kernel_function(q_hbm, k_hbm, v_hbm, o_hbm, qb, kb, vb, ob, rsem, tsem, wsem):
        pairs = ((q_hbm, qb), (k_hbm, kb), (v_hbm, vb))

        def read(c, j):
            src, dst = pairs[j]
            rows = pl.ds(c * _CHUNK, _CHUNK)
            return pltpu.make_async_copy(src.at[rows], dst.at[rows], rsem.at[j, c])

        def tail_read(i, j, start, size):
            src, dst = pairs[j]
            rows = pl.ds(start, size)
            return pltpu.make_async_copy(src.at[rows], dst.at[rows], tsem.at[i])

        def write(c):
            rows = pl.ds(c * _CHUNK, _CHUNK)
            return pltpu.make_async_copy(ob.at[rows], o_hbm.at[rows], wsem.at[c])

        tail = [
            tail_read(0, 0, h0, n - h0),
            tail_read(1, 1, h0, n - h0),
            tail_read(2, 2, h0, n - h0 - _LAST),
            tail_read(3, 2, n - _LAST, _LAST),
        ]
        first_write = pltpu.make_async_copy(
            ob.at[pl.ds(0, h0)], o_hbm.at[pl.ds(0, h0)], wsem.at[0]
        )

        for c in range(_SWITCH):
            for j in range(3):
                read(c, j).start()
        for t in tail:
            t.start()

        def chunk(c, _):
            @pl.when(c < _SWITCH)
            def _():
                for j in range(3):
                    read(c, j).wait()

            @pl.when(c == _SWITCH)
            def _():
                for t in tail[:3]:
                    t.wait()
                first_write.start()
                tail[3].wait()

            def group(g, _):
                base = c * _CHUNK + g * _GROUP
                for i in range(_GROUP):
                    x = base + i
                    ob[x] = _attend(qb[x], kb[x], vb[x]).astype(ob.dtype)

            lax.fori_loop(0, _CHUNK // _GROUP, group, None)

            @pl.when(c >= _SWITCH)
            def _():
                write(c).start()

        lax.fori_loop(0, nc, chunk, None)
        first_write.wait()
        for c in range(_SWITCH, nc):
            write(c).wait()

    out = pl.pallas_call(
        kernel_function,
        in_specs=[pl.BlockSpec(memory_space=pl.ANY)] * 3,
        out_specs=pl.BlockSpec(memory_space=pl.ANY),
        out_shape=jax.ShapeDtypeStruct((n, sq, d), q.dtype),
        scratch_shapes=[
            pltpu.VMEM((n, sq, d), q.dtype),
            pltpu.VMEM((n, sk, d), k.dtype),
            pltpu.VMEM((n, sk, d), v.dtype),
            pltpu.VMEM((n, sq, d), q.dtype),
            pltpu.SemaphoreType.DMA((3, _SWITCH)),
            pltpu.SemaphoreType.DMA((4,)),
            pltpu.SemaphoreType.DMA((nc,)),
        ],
        compiler_params=pltpu.CompilerParams(vmem_limit_bytes=124 * 2**20),
    )(q.reshape(n, sq, d), k.reshape(n, sk, d), v.reshape(n, sk, d))
    return out.reshape(b, h, sq, d)
```

```python
import jax
import jax.numpy as jnp
from jax import lax
import jax.experimental.pallas as pl
import jax.experimental.pallas.tpu as pltpu

_LOG2E = 1.4426950408889634

_GROUP = 8

_READS = (
    (0, 0, 32), (1, 0, 16), (2, 0, 8), (2, 8, 32), (1, 16, 40), (0, 32, 80),
    (2, 32, 48), (1, 40, 64), (2, 48, 72), (1, 64, 112), (2, 72, 96),
    (0, 80, 120), (2, 96, 144), (1, 112, 160), (0, 120, 152), (0, 152, 200),
    (2, 144, 184), (1, 160, 208), (2, 184, 256), (0, 200, 256), (1, 208, 252),
    (1, 252, 256),
)
_SWITCH = 208

_PIECE_ROWS = 64
_PIECES = 64
_REGIONS = ((0, 16), (16, 20), (20, 24))
_WRITES = ((208, 0, 0, 64), (240, 1, 0, 32), (248, 1, 32, 64), (256, 2, 0, 64))


def _attend(q, k, v):
    scale = (q.shape[-1] ** -0.5) * _LOG2E
    s = lax.dot_general(
        q, k, (((1,), (1,)), ((), ())), preferred_element_type=jnp.float32
    )
    m = jnp.max(s, axis=-1, keepdims=True)
    p = jnp.exp2((s - m) * scale)
    l = jnp.sum(p, axis=-1, keepdims=True)
    o = jnp.dot(p.astype(v.dtype), v, preferred_element_type=jnp.float32)
    r = pl.reciprocal(l, approx=True)
    r = r * (2.0 - l * r)
    return o * r


@jax.jit
def pallas_standalone__mha_softmax__near_ridge_kernel(
    q: jax.Array,
    k: jax.Array,
    v: jax.Array,
):
    b, h, sq, d = q.shape
    sk = k.shape[2]
    n = b * h
    blocks = _REGIONS[-1][1]
    per_head = sq // _PIECE_ROWS
    assert n == _WRITES[-1][0] and n * per_head == blocks * _PIECES

    def kernel_function(q_hbm, k_hbm, v_hbm, o_hbm, qb, kb, vb, ob, rsem, wsem):
        operands = ((q_hbm, qb), (k_hbm, kb), (v_hbm, vb))

        def read(i):
            a, start, end = _READS[i]
            src, dst = operands[a]
            heads = pl.ds(start, end - start)
            return pltpu.make_async_copy(src.at[heads], dst.at[heads], rsem.at[i])

        def region(r):
            return pl.ds(_REGIONS[r][0], _REGIONS[r][1] - _REGIONS[r][0])

        def start_writes(done):
            for at, r, lo, hi in _WRITES:
                if at == done:
                    for i in range(lo, hi):
                        pltpu.make_async_copy(
                            ob.at[region(r), i], o_hbm.at[region(r), i], wsem.at[r]
                        ).start()

        for i in range(len(_READS)):
            read(i).start()

        last = len(_READS) - 1
        waits = {}
        for i, (_, start, _) in enumerate(_READS[:last]):
            waits.setdefault(min(start // _GROUP * _GROUP, _SWITCH), []).append(i)
        events = sorted(set(waits) | {w[0] for w in _WRITES if w[0] < n})

        def group(g, carry):
            first = g * _GROUP
            for at in events:

                @pl.when(first == at)
                def _():
                    for i in waits.get(at, ()):
                        read(i).wait()
                    start_writes(at)
                    if at == _SWITCH:
                        read(last).wait()

            for x in range(_GROUP):
                head = first + x
                o = _attend(qb[head], kb[head], vb[head]).astype(ob.dtype)
                for j in range(per_head):
                    t = head * per_head + j
                    ob[t // _PIECES, t % _PIECES] = o[
                        j * _PIECE_ROWS : (j + 1) * _PIECE_ROWS
                    ]
            return carry

        lax.fori_loop(0, n // _GROUP, group, None)

        start_writes(n)
        for r in range(len(_REGIONS)):
            pltpu.make_async_copy(
                ob.at[region(r)], o_hbm.at[region(r)], wsem.at[r]
            ).wait()

    out_view = (blocks, _PIECES, _PIECE_ROWS, d)
    out = pl.pallas_call(
        kernel_function,
        in_specs=[pl.BlockSpec(memory_space=pl.ANY)] * 3,
        out_specs=pl.BlockSpec(memory_space=pl.ANY),
        out_shape=jax.ShapeDtypeStruct(out_view, q.dtype),
        scratch_shapes=[
            pltpu.VMEM((n, sq, d), q.dtype),
            pltpu.VMEM((n, sk, d), k.dtype),
            pltpu.VMEM((n, sk, d), v.dtype),
            pltpu.VMEM(out_view, q.dtype),
            pltpu.SemaphoreType.DMA((len(_READS),)),
            pltpu.SemaphoreType.DMA((len(_REGIONS),)),
        ],
        compiler_params=pltpu.CompilerParams(vmem_limit_bytes=124 * 2**20),
    )(q.reshape(n, sq, d), k.reshape(n, sk, d), v.reshape(n, sk, d))
    return out.reshape(b, h, sq, d)
```

```python
import jax
import jax.numpy as jnp
from jax import lax
import jax.experimental.pallas as pl
import jax.experimental.pallas.tpu as pltpu

_LOG2E = 1.4426950408889634

_GROUP = 8

_READ_BOUNDS = (8, 16, 24, 32, 48, 64, 80, 96, 120, 144, 176, 208)
_TAIL_HEADS = 3

_PIECE_ROWS = 64
_PIECES = 64
_REGIONS = ((0, 16), (16, 20), (20, 24))
_WRITES = ((208, 0, 0, 64), (240, 1, 0, 32), (248, 1, 32, 64), (256, 2, 0, 64))


def _attend(q, k, v):
    scale = (q.shape[-1] ** -0.5) * _LOG2E
    s = lax.dot_general(
        q, k, (((1,), (1,)), ((), ())), preferred_element_type=jnp.float32
    )
    m = jnp.max(s, axis=-1, keepdims=True)
    p = jnp.exp2((s - m) * scale)
    l = jnp.sum(p, axis=-1, keepdims=True)
    o = jnp.dot(p.astype(v.dtype), v, preferred_element_type=jnp.float32)
    r = pl.reciprocal(l, approx=True)
    r = r * (2.0 - l * r)
    return o * r


def _dispatch(value, keys, handler):
    if len(keys) == 1:
        pl.when(value == keys[0])(lambda: handler(keys[0]))
    else:
        half = len(keys) // 2
        lax.cond(
            value < keys[half],
            lambda: _dispatch(value, keys[:half], handler),
            lambda: _dispatch(value, keys[half:], handler),
        )


@jax.jit
def pallas_standalone__mha_softmax__near_ridge_kernel(
    q: jax.Array,
    k: jax.Array,
    v: jax.Array,
):
    b, h, sq, d = q.shape
    sk = k.shape[2]
    n = b * h
    blocks = _REGIONS[-1][1]
    per_head = sq // _PIECE_ROWS
    assert n == _WRITES[-1][0] and n * per_head == blocks * _PIECES

    starts = (0,) + _READ_BOUNDS
    ends = _READ_BOUNDS + (n,)
    tail = len(starts)
    chunk_at = {first: c for c, first in enumerate(starts)}
    events = sorted(set(starts) | {w[0] for w in _WRITES if w[0] < n})

    def kernel_function(q_hbm, k_hbm, v_hbm, o_hbm, qb, kb, vb, ob, sems):
        def reads(c):
            if c == tail:
                spans = [(v_hbm, vb, n - _TAIL_HEADS, n)]
            else:
                v_end = min(ends[c], n - _TAIL_HEADS)
                spans = [
                    (q_hbm, qb, starts[c], ends[c]),
                    (k_hbm, kb, starts[c], ends[c]),
                    (v_hbm, vb, starts[c], v_end),
                ]
            return [
                pltpu.make_async_copy(
                    src.at[pl.ds(lo, hi - lo)],
                    dst.at[pl.ds(lo, hi - lo)],
                    sems.at[c % 2],
                )
                for src, dst, lo, hi in spans
            ]

        def start_reads(c):
            for copy in reads(c):
                copy.start()

        def wait_reads(c):
            for copy in reads(c):
                copy.wait()

        write_sem = sems.at[(tail - 1) % 2]

        def start_writes(done):
            for at, r, lo, hi in _WRITES:
                if at == done:
                    region = pl.ds(_REGIONS[r][0], _REGIONS[r][1] - _REGIONS[r][0])
                    for i in range(lo, hi):
                        pltpu.make_async_copy(
                            ob.at[region, i], o_hbm.at[region, i], write_sem
                        ).start()

        def before_head(first):
            if first in chunk_at:
                c = chunk_at[first]
                wait_reads(c)
                if c + 2 <= tail:
                    start_reads(c + 2)
            start_writes(first)
            if first == starts[-1]:
                wait_reads(tail)

        def group(g, carry):
            first = g * _GROUP
            _dispatch(first, events, before_head)
            for x in range(_GROUP):
                head = first + x
                o = _attend(qb[head], kb[head], vb[head]).astype(ob.dtype)
                for j in range(per_head):
                    t = head * per_head + j
                    ob[t // _PIECES, t % _PIECES] = o[
                        j * _PIECE_ROWS : (j + 1) * _PIECE_ROWS
                    ]
            return carry

        start_reads(0)
        start_reads(1)
        lax.fori_loop(0, n // _GROUP, group, None)
        start_writes(n)
        pltpu.make_async_copy(ob, o_hbm, write_sem).wait()

    out_view = (blocks, _PIECES, _PIECE_ROWS, d)
    out = pl.pallas_call(
        kernel_function,
        in_specs=[pl.BlockSpec(memory_space=pl.ANY)] * 3,
        out_specs=pl.BlockSpec(memory_space=pl.ANY),
        out_shape=jax.ShapeDtypeStruct(out_view, q.dtype),
        scratch_shapes=[
            pltpu.VMEM((n, sq, d), q.dtype),
            pltpu.VMEM((n, sk, d), k.dtype),
            pltpu.VMEM((n, sk, d), v.dtype),
            pltpu.VMEM(out_view, q.dtype),
            pltpu.SemaphoreType.DMA((2,)),
        ],
        compiler_params=pltpu.CompilerParams(vmem_limit_bytes=124 * 2**20),
    )(q.reshape(n, sq, d), k.reshape(n, sk, d), v.reshape(n, sk, d))
    return out.reshape(b, h, sq, d)
```

```python
import jax
import jax.numpy as jnp
from jax import lax
import jax.experimental.pallas as pl
import jax.experimental.pallas.tpu as pltpu

_LOG2E = 1.4426950408889634

_GROUP = 8

_READ_BOUNDS = (8, 16, 24, 32, 48, 64, 80, 96, 120, 144, 176, 208)
_TAIL_HEADS = 3

_PIECE_ROWS = 64
_PIECES = 64
_REGIONS = ((0, 8), (8, 14), (14, 20), (20, 24))
_WRITES = (
    (208, 0, 0, 64),
    (216, 1, 0, 26),
    (224, 1, 26, 51),
    (232, 1, 51, 64),
    (232, 2, 0, 15),
    (240, 2, 15, 48),
    (248, 2, 48, 64),
    (256, 3, 0, 64),
)


def _attend(q, k, v):
    scale = (q.shape[-1] ** -0.5) * _LOG2E
    s = lax.dot_general(
        q, k, (((1,), (1,)), ((), ())), preferred_element_type=jnp.float32
    )
    m = jnp.max(s, axis=-1, keepdims=True)
    p = jnp.exp2((s - m) * scale)
    l = jnp.sum(p, axis=-1, keepdims=True)
    o = jnp.dot(p.astype(v.dtype), v, preferred_element_type=jnp.float32)
    r = pl.reciprocal(l, approx=True)
    r = r * (2.0 - l * r)
    return o * r


def _dispatch(value, keys, handler):
    if len(keys) == 1:
        pl.when(value == keys[0])(lambda: handler(keys[0]))
    else:
        half = len(keys) // 2
        lax.cond(
            value < keys[half],
            lambda: _dispatch(value, keys[:half], handler),
            lambda: _dispatch(value, keys[half:], handler),
        )


@jax.jit
def pallas_standalone__mha_softmax__near_ridge_kernel(
    q: jax.Array,
    k: jax.Array,
    v: jax.Array,
):
    b, h, sq, d = q.shape
    sk = k.shape[2]
    n = b * h
    blocks = _REGIONS[-1][1]
    per_head = sq // _PIECE_ROWS
    assert _TAIL_HEADS <= _GROUP and n * per_head == blocks * _PIECES
    for at, r, _, _ in _WRITES:
        assert _REGIONS[r][1] * _PIECES <= at * per_head

    starts = (0,) + _READ_BOUNDS
    ends = _READ_BOUNDS + (n,)
    tail = len(starts)
    chunk_at = {first: c for c, first in enumerate(starts)}
    last_group = n - _GROUP
    events = sorted(
        set(starts) | {w[0] for w in _WRITES if w[0] < n} | {last_group}
    )

    def kernel_function(q_hbm, k_hbm, v_hbm, o_hbm, qb, kb, vb, ob, sems):
        def reads(c):
            if c == tail:
                spans = [(v_hbm, vb, n - _TAIL_HEADS, n)]
            else:
                v_end = min(ends[c], n - _TAIL_HEADS)
                spans = [
                    (q_hbm, qb, starts[c], ends[c]),
                    (k_hbm, kb, starts[c], ends[c]),
                    (v_hbm, vb, starts[c], v_end),
                ]
            return [
                pltpu.make_async_copy(
                    src.at[pl.ds(lo, hi - lo)],
                    dst.at[pl.ds(lo, hi - lo)],
                    sems.at[c % 2],
                )
                for src, dst, lo, hi in spans
            ]

        def start_reads(c):
            for copy in reads(c):
                copy.start()

        def wait_reads(c):
            for copy in reads(c):
                copy.wait()

        write_sem = sems.at[(tail - 1) % 2]

        def start_writes(done):
            for at, r, lo, hi in _WRITES:
                if at == done:
                    region = pl.ds(_REGIONS[r][0], _REGIONS[r][1] - _REGIONS[r][0])
                    for i in range(lo, hi):
                        pltpu.make_async_copy(
                            ob.at[region, i], o_hbm.at[region, i], write_sem
                        ).start()

        def before_head(first):
            if first in chunk_at:
                c = chunk_at[first]
                wait_reads(c)
                if c + 2 <= tail:
                    start_reads(c + 2)
            start_writes(first)
            if first == last_group:
                wait_reads(tail)

        def group(g, carry):
            first = g * _GROUP
            _dispatch(first, events, before_head)
            for x in range(_GROUP):
                head = first + x
                o = _attend(qb[head], kb[head], vb[head]).astype(ob.dtype)
                for j in range(per_head):
                    t = head * per_head + j
                    ob[t // _PIECES, t % _PIECES] = o[
                        j * _PIECE_ROWS : (j + 1) * _PIECE_ROWS
                    ]
            return carry

        start_reads(0)
        start_reads(1)
        lax.fori_loop(0, n // _GROUP, group, None)
        start_writes(n)
        pltpu.make_async_copy(ob, o_hbm, write_sem).wait()

    out_view = (blocks, _PIECES, _PIECE_ROWS, d)
    out = pl.pallas_call(
        kernel_function,
        in_specs=[pl.BlockSpec(memory_space=pl.ANY)] * 3,
        out_specs=pl.BlockSpec(memory_space=pl.ANY),
        out_shape=jax.ShapeDtypeStruct(out_view, q.dtype),
        scratch_shapes=[
            pltpu.VMEM((n, sq, d), q.dtype),
            pltpu.VMEM((n, sk, d), k.dtype),
            pltpu.VMEM((n, sk, d), v.dtype),
            pltpu.VMEM(out_view, q.dtype),
            pltpu.SemaphoreType.DMA((2,)),
        ],
        compiler_params=pltpu.CompilerParams(vmem_limit_bytes=124 * 2**20),
    )(q.reshape(n, sq, d), k.reshape(n, sk, d), v.reshape(n, sk, d))
    return out.reshape(b, h, sq, d)
```
